```python
import jax
import jax.numpy as jnp

def _softmax(x, axis=-1):
    return jax.nn.softmax(x, axis=axis)
def _gelu(x):
    return jax.nn.gelu(x, approximate=True)
def _silu(x):
    return jax.nn.silu(x)
def _sigmoid(x):
    return jax.nn.sigmoid(x)
def _layernorm(x, axis=-1, eps=1e-5):
    m = jnp.mean(x, axis=axis, keepdims=True)
    v = jnp.var(x, axis=axis, keepdims=True)
    return (x - m) / jnp.sqrt(v + eps)
def _scatter_add(tgt, idx, src, axis=0):
    return tgt.at[idx].add(src)
def _segment_sum(src, seg, n):
    return jax.ops.segment_sum(src, seg, n)
class _Rng:
    def __init__(self, key):
        self._k = key
    def _next(self):
        self._k, sub = jax.random.split(self._k)
        return sub
    def normal(self, shape):
        return jax.random.normal(self._next(), shape, dtype=jnp.bfloat16)
    def randint(self, lo, hi, shape):
        return jax.random.randint(self._next(), shape, lo, hi, dtype=jnp.int32)
    def uniform(self, shape, lo=0.0, hi=1.0):
        return jax.random.uniform(self._next(), shape, jnp.bfloat16, lo, hi)
    def permutation(self, n):
        return jax.random.permutation(self._next(), n)


kernel_name = 'standalone__cross_network_dcn__recsys'

def setup_inputs():
    _rng = _Rng(jax.random.key(int.from_bytes(__import__("os").urandom(4), "little")))
    _w = (lambda a: (lambda t: t.astype(jnp.bfloat16) if jnp.issubdtype(t.dtype, jnp.floating) else t)(jnp.asarray(a)))
    B, F, D, L = 16384, 100, 16, 6
    Din = min(F * D, 1024)
    return {
        "x0": _w((lambda *s: _rng.normal(s) * 0.05)(B, Din)),
        "ws": _w((lambda *s: _rng.normal(s) * 0.05)(L, Din, Din) * (Din ** -0.5)),
        "bs": _w((lambda *s: _rng.normal(s) * 0.05)(L, Din) * 0.01),
    }

def reference(x0, ws, bs):
    x = x0
    L = ws.shape[0]
    for l in range(L):
        proj = jnp.einsum('bd,de->be', x, ws[l]) + bs[l]
        x = x0 * proj + x
    return x
```

```python
import jax
import jax.numpy as jnp
from jax.experimental import pallas as pl
from jax.experimental.pallas import tpu as pltpu

F32, BF16, U32 = jnp.float32, jnp.bfloat16, jnp.uint32
NB = 4
ORDER = (3, 4, 1, 2, 5, 6, 7)
TM = 512
CR, CC = 16, 128


def _quad(X):
    n = len(X) // 2
    return ([r[:n] for r in X[:n]], [r[n:] for r in X[:n]],
            [r[:n] for r in X[n:]], [r[n:] for r in X[n:]])


def _add(X, Y):
    return [[a + b for a, b in zip(r, s)] for r, s in zip(X, Y)]


def _sub(X, Y):
    return [[a - b for a, b in zip(r, s)] for r, s in zip(X, Y)]


def _lhs(A, m):
    A12, A11, A22, A21 = _quad(A)
    return {1: lambda: _add(A11, A22), 2: lambda: _add(A21, A22),
            3: lambda: A11, 4: lambda: A22, 5: lambda: _add(A11, A12),
            6: lambda: _sub(A21, A11), 7: lambda: _sub(A12, A22)}[m]()


def _rhs(B, m):
    B21, B22, B11, B12 = _quad(B)
    return {1: lambda: _add(B11, B22), 2: lambda: B11,
            3: lambda: _sub(B12, B22), 4: lambda: _sub(B21, B11),
            5: lambda: B22, 6: lambda: _add(B11, B12),
            7: lambda: _add(B21, B22)}[m]()


def _matmul(A, weight, k0):
    if len(A) == 1:
        return [[jnp.dot(A[0][0].astype(BF16), weight(k0), preferred_element_type=F32)]]
    stride = 7 ** (len(A).bit_length() - 2)
    M = {}
    for i, m in enumerate(ORDER):
        M[m] = _matmul(_lhs(A, m), weight, k0 + i * stride)
        if m == 1:
            U, V = _add(M[1], M[4]), _add(M[1], M[3])
        elif m == 2:
            C21, V = _add(M[2], M[4]), _sub(V, M[2])
        elif m == 5:
            C12, U = _add(M[3], M[5]), _sub(U, M[5])
        elif m == 6:
            C22 = _add(V, M[6])
        elif m == 7:
            C11 = _add(U, M[7])
    return [a + b for a, b in zip(C11, C12)] + [a + b for a, b in zip(C21, C22)]


def _kernel(x0_ref, w_hbm, b_ref, o_ref, c_ref, w_ref, sem):
    L, D, _ = w_ref.shape
    H, h = D // NB, x0_ref.shape[0] // NB

    def blk(ref, i, j):
        return ref.at[i * h:(i + 1) * h, j * H:(j + 1) * H]

    def dma(l):
        return pltpu.make_async_copy(w_hbm.at[l], w_ref.at[l], sem.at[l])

    def weight_sums(l, g, r, cc):
        words = [[pltpu.bitcast(
            w_ref[l, pl.ds(i * H + r * CR, CR), j * H + cc * CC:j * H + (cc + 1) * CC], U32)
            for j in range(NB)] for i in range(NB)]
        terms = []
        for p in range(2):
            Bm = [[pltpu.unpack_elementwise(u, index=p, packed_dtype=BF16, unpacked_dtype=F32)
                   for u in row] for row in words]
            outer = _rhs(Bm, ORDER[g])
            terms.append([_rhs(outer, m)[0][0] for m in ORDER])
        for k in range(7):
            c_ref[l, 7 * g + k, pl.ds(r * (CR // 2), CR // 2), cc * CC:(cc + 1) * CC] = (
                pltpu.pack_elementwise([terms[0][k], terms[1][k]], packed_dtype=BF16))

    @pl.when(pl.program_id(0) == 0)
    def _():
        for l in range(min(2, L)):
            dma(l).start()

        @pl.loop(0, L)
        def _(l):
            dma(l).wait()

            @pl.when(l + 2 < L)
            def _():
                dma(l + 2).start()

            for g in range(7):
                @pl.loop(0, H // CR)
                def _(r):
                    for cc in range(H // CC):
                        weight_sums(l, g, r, cc)

    X = [[blk(x0_ref, i, j)[...].astype(F32) for j in range(NB)] for i in range(NB)]
    for l in range(L):
        C = _matmul(X, lambda k: pltpu.bitcast(c_ref[l, k], BF16), 0)
        b = b_ref[l:l + 1, :].astype(F32)
        X = [[blk(x0_ref, i, j)[...].astype(F32) * (C[i][j] + b[:, j * H:(j + 1) * H]) + X[i][j]
              for j in range(NB)] for i in range(NB)]
    for i in range(NB):
        for j in range(NB):
            blk(o_ref, i, j)[...] = X[i][j].astype(o_ref.dtype)


@jax.jit
def pallas_standalone__cross_network_dcn__recsys_kernel(x0, ws, bs):
    B, D = x0.shape
    L = ws.shape[0]
    assert B % TM == 0 and D % (NB * CC) == 0
    return pl.pallas_call(
        _kernel,
        grid=(B // TM,),
        in_specs=[pl.BlockSpec((TM, D), lambda i: (i, 0)),
                  pl.BlockSpec(memory_space=pl.ANY),
                  pl.BlockSpec((L, D), lambda i: (0, 0))],
        out_specs=pl.BlockSpec((TM, D), lambda i: (i, 0)),
        out_shape=jax.ShapeDtypeStruct((B, D), x0.dtype),
        scratch_shapes=[pltpu.VMEM((L, 49, D // NB // 2, D // NB), U32),
                        pltpu.VMEM((L, D, D), BF16),
                        pltpu.SemaphoreType.DMA((L,))],
        compiler_params=pltpu.CompilerParams(
            dimension_semantics=("arbitrary",),
            vmem_limit_bytes=100 * 2**20,
            flags={"XLA_TPU_FORCE_LP_LLO_SCHEDULER": True}),
    )(x0, ws, bs)
```

```python
import jax
import jax.numpy as jnp
from jax.experimental import pallas as pl
from jax.experimental.pallas import tpu as pltpu

F32, BF16, U32 = jnp.float32, jnp.bfloat16, jnp.uint32
NB = 4
ORDER = (3, 4, 1, 2, 5, 6, 7)
TM = 768
HEAD = 256
CR, CC = 16, 128


def _quad(X):
    n = len(X) // 2
    return ([r[:n] for r in X[:n]], [r[n:] for r in X[:n]],
            [r[:n] for r in X[n:]], [r[n:] for r in X[n:]])


def _add(X, Y):
    return [[a + b for a, b in zip(r, s)] for r, s in zip(X, Y)]


def _sub(X, Y):
    return [[a - b for a, b in zip(r, s)] for r, s in zip(X, Y)]


def _lhs(A, m):
    A12, A11, A22, A21 = _quad(A)
    return {1: lambda: _add(A11, A22), 2: lambda: _add(A21, A22),
            3: lambda: A11, 4: lambda: A22, 5: lambda: _add(A11, A12),
            6: lambda: _sub(A21, A11), 7: lambda: _sub(A12, A22)}[m]()


def _rhs(B, m):
    B21, B22, B11, B12 = _quad(B)
    return {1: lambda: _add(B11, B22), 2: lambda: B11,
            3: lambda: _sub(B12, B22), 4: lambda: _sub(B21, B11),
            5: lambda: B22, 6: lambda: _add(B11, B12),
            7: lambda: _add(B21, B22)}[m]()


def _matmul(A, weight, k0):
    if len(A) == 1:
        return [[jnp.dot(A[0][0].astype(BF16), weight(k0), preferred_element_type=F32)]]
    stride = 7 ** (len(A).bit_length() - 2)
    M = {}
    for i, m in enumerate(ORDER):
        M[m] = _matmul(_lhs(A, m), weight, k0 + i * stride)
        if m == 1:
            U, V = _add(M[1], M[4]), _add(M[1], M[3])
        elif m == 2:
            C21, V = _add(M[2], M[4]), _sub(V, M[2])
        elif m == 5:
            C12, U = _add(M[3], M[5]), _sub(U, M[5])
        elif m == 6:
            C22 = _add(V, M[6])
        elif m == 7:
            C11 = _add(U, M[7])
    return [a + b for a, b in zip(C11, C12)] + [a + b for a, b in zip(C21, C22)]


def _kernel(x_hbm, w_hbm, b_ref, o_hbm,
            c_ref, w_ref, xin, xout, xp, xs, zero_ref, wsem, isem, osem, psem):
    L, D, _ = w_ref.shape
    H, h = D // NB, TM // NB
    NT = (x_hbm.shape[0] - HEAD) // TM

    def blk(ref, i, j):
        return ref.at[i * h:(i + 1) * h, j * H:(j + 1) * H]

    def rows(t, off, n):
        return pl.ds(pl.multiple_of(HEAD + t * TM + off, 64), n)

    def w_copy(l):
        return pltpu.make_async_copy(w_hbm.at[l], w_ref.at[l], wsem.at[l])

    def x_copy(t):
        return pltpu.make_async_copy(x_hbm.at[rows(t, 0, TM)], xin.at[t & 1], isem.at[t & 1])

    def out_wait(slot):
        pltpu.make_async_copy(xout.at[slot], xout.at[slot], osem.at[slot]).wait()

    head_in = pltpu.make_async_copy(x_hbm.at[0:HEAD], xp, psem.at[0])
    head_out = pltpu.make_async_copy(xp, o_hbm.at[0:HEAD], psem.at[1])

    def weight_sums(l, g, r, cc, zero):
        words = [[pltpu.bitcast(
            w_ref[l, i * H + r * CR:i * H + (r + 1) * CR, j * H + cc * CC:j * H + (cc + 1) * CC],
            U32) for j in range(NB)] for i in range(NB)]
        shift, mask = zero | jnp.uint32(16), zero | jnp.uint32(0xFFFF0000)
        terms = []
        for odd in range(2):
            Bm = [[pltpu.bitcast((u & mask) if odd else (u << shift), F32) for u in row]
                  for row in words]
            outer = _rhs(Bm, ORDER[g])
            terms.append([_rhs(outer, m)[0][0] for m in ORDER])
        for k in range(7):
            c_ref[l, 7 * g + k, r * (CR // 2):(r + 1) * (CR // 2), cc * CC:(cc + 1) * CC] = (
                pltpu.pack_elementwise([terms[0][k], terms[1][k]], packed_dtype=BF16))

    head_in.start()
    w_copy(0).start()
    zero_ref[...] = jnp.zeros(zero_ref.shape, U32)
    head_in.wait()
    xs[...] = xp[...].astype(F32)

    @pl.loop(0, L)
    def _(l):
        w_copy(l).wait()

        @pl.when(l + 1 < L)
        def _():
            w_copy(l + 1).start()

        @pl.when(l + 1 == L)
        def _():
            x_copy(0).start()

        b = b_ref[...].astype(F32)
        b = jnp.sum(jnp.where(jax.lax.broadcasted_iota(jnp.int32, b.shape, 0) == l, b, 0.0),
                    axis=0, keepdims=True)
        xb, zeros = xs[...].astype(BF16), zero_ref[...]
        work = [(g, r, cc) for r in range(H // CR) for cc in range(H // CC) for g in range(7)]
        parts = 2 * (D // CC)
        for j in range(D // CC):
            cols = slice(j * CC, (j + 1) * CC)
            ps = [jnp.dot(xb[:, k * 2 * H:(k + 1) * 2 * H], w_ref[l, k * 2 * H:(k + 1) * 2 * H, cols],
                          preferred_element_type=F32) for k in range(2)]
            xs[:, cols] = xp[:, cols].astype(F32) * (ps[0] + ps[1] + b[:, cols]) + xs[:, cols]
            for k in range(2):
                u = 2 * j + k
                todo = work[u * len(work) // parts:(u + 1) * len(work) // parts]
                for q, (g, r, cc) in enumerate(todo):
                    s = 8 * (q * (HEAD // 8) // len(todo))
                    weight_sums(l, g, r, cc, pltpu.bitcast(ps[k][s:s + 8], U32) & zeros)

    xp[...] = xs[...].astype(xp.dtype)
    head_out.start()

    @pl.loop(0, NT)
    def _(t):
        slot = t & 1
        x_copy(t).wait()

        @pl.when(t >= 2)
        def _():
            out_wait(slot)

        @pl.when(t + 1 < NT)
        def _():
            x_copy(t + 1).start()

        x0_ref, o_ref = xin.at[slot], xout.at[slot]
        X = [[blk(x0_ref, i, j)[...].astype(F32) for j in range(NB)] for i in range(NB)]
        for l in range(L):
            C = _matmul(X, lambda k: pltpu.bitcast(c_ref[l, k], BF16), 0)
            b = b_ref[l:l + 1, :].astype(F32)
            X = [[blk(x0_ref, i, j)[...].astype(F32) * (C[i][j] + b[:, j * H:(j + 1) * H]) + X[i][j]
                  for j in range(NB)] for i in range(NB)]
        for I, J in ((1, 0), (0, 1), (1, 1), (0, 0)):
            for i in range(2 * I, 2 * I + 2):
                for j in range(2 * J, 2 * J + 2):
                    blk(o_ref, i, j)[...] = X[i][j].astype(o_ref.dtype)
            cols = slice(J * 2 * H, (J + 1) * 2 * H)
            pltpu.make_async_copy(o_ref.at[I * 2 * h:(I + 1) * 2 * h, cols],
                                  o_hbm.at[rows(t, I * 2 * h, 2 * h), cols],
                                  osem.at[slot]).start()

    head_out.wait()
    out_wait(0)
    out_wait(1)


@jax.jit
def pallas_standalone__cross_network_dcn__recsys_kernel(x0, ws, bs):
    B, D = x0.shape
    L = ws.shape[0]
    assert (B - HEAD) % TM == 0 and B - HEAD >= 2 * TM and D % (NB * CC) == 0
    assert x0.dtype == BF16 and ws.dtype == BF16
    return pl.pallas_call(
        _kernel,
        in_specs=[pl.BlockSpec(memory_space=pl.ANY),
                  pl.BlockSpec(memory_space=pl.ANY),
                  pl.BlockSpec(memory_space=pltpu.VMEM)],
        out_specs=pl.BlockSpec(memory_space=pl.ANY),
        out_shape=jax.ShapeDtypeStruct((B, D), x0.dtype),
        scratch_shapes=[pltpu.VMEM((L, 49, D // NB // 2, D // NB), U32),
                        pltpu.VMEM((L, D, D), BF16),
                        pltpu.VMEM((2, TM, D), BF16),
                        pltpu.VMEM((2, TM, D), BF16),
                        pltpu.VMEM((HEAD, D), BF16),
                        pltpu.VMEM((HEAD, D), F32),
                        pltpu.VMEM((8, CC), U32),
                        pltpu.SemaphoreType.DMA((L,)),
                        pltpu.SemaphoreType.DMA((2,)),
                        pltpu.SemaphoreType.DMA((2,)),
                        pltpu.SemaphoreType.DMA((2,))],
        compiler_params=pltpu.CompilerParams(
            vmem_limit_bytes=100 * 2**20,
            flags={"XLA_TPU_FORCE_LP_LLO_SCHEDULER": True}),
    )(x0, ws, bs)
```

```python
import functools

import jax
import jax.numpy as jnp
from jax.experimental import pallas as pl
from jax.experimental.pallas import tpu as pltpu

F32 = jnp.float32


def _kernel(x_hbm, w_hbm, b_ref, o_hbm, w_ref, xin, xout, xp, xs,
            wsem, w0sem, isem, osem, psem, *, out_parts):
    L, D, _ = w_ref.shape
    HEAD, TM = xp.shape[0], xin.shape[1]
    NT = (x_hbm.shape[0] - HEAD) // TM
    W0 = w0sem.shape[0]

    def rows(t):
        return pl.ds(pl.multiple_of(HEAD + t * TM, 64), TM)

    def part(j, n):
        return slice(j * (D // n), (j + 1) * (D // n))

    def w_copy(l):
        return pltpu.make_async_copy(w_hbm.at[l], w_ref.at[l], wsem.at[l])

    def w0_copy(j):
        return pltpu.make_async_copy(w_hbm.at[0, :, part(j, W0)], w_ref.at[0, :, part(j, W0)],
                                     w0sem.at[j])

    def x_copy(t):
        return pltpu.make_async_copy(x_hbm.at[rows(t)], xin.at[t & 1], isem.at[t & 1])

    def out_wait(slot):
        pltpu.make_async_copy(xout.at[slot], xout.at[slot], osem.at[slot]).wait()

    head_in = pltpu.make_async_copy(x_hbm.at[0:HEAD], xp, psem.at[0])
    head_out = pltpu.make_async_copy(xp, o_hbm.at[0:HEAD], psem.at[1])

    ahead = [w0_copy(j) for j in range(W0)] + [w_copy(1)]
    head_in.start()
    ahead[0].start()
    head_in.wait()
    ahead[1].start()
    for j in range(W0):
        cols = part(j, W0)
        ahead[j].wait()
        if j + 2 < len(ahead):
            ahead[j + 2].start()
        x0 = xp[:, cols].astype(F32)
        proj = jnp.dot(xp[...], w_ref[0, :, cols], preferred_element_type=F32)
        xs[:, cols] = x0 * (proj + b_ref[0:1, cols].astype(F32)) + x0

    @pl.loop(1, L)
    def _(l):
        w_copy(l).wait()

        @pl.when(l + 1 < L)
        def _():
            w_copy(l + 1).start()

        @pl.when(l + 1 == L)
        def _():
            x_copy(0).start()

        b = b_ref[...].astype(F32)
        b = jnp.sum(jnp.where(jax.lax.broadcasted_iota(jnp.int32, b.shape, 0) == l, b, 0.0),
                    axis=0, keepdims=True)
        x = xs[...]
        proj = jnp.dot(x.astype(w_ref.dtype), w_ref[l], preferred_element_type=F32)
        xs[...] = xp[...].astype(F32) * (proj + b) + x

    xp[...] = xs[...].astype(xp.dtype)
    head_out.start()

    @pl.loop(0, NT)
    def _(t):
        slot = t & 1
        x_copy(t).wait()

        @pl.when(t >= 2)
        def _():
            out_wait(slot)

        @pl.when(t + 1 < NT)
        def _():
            x_copy(t + 1).start()

        x0_ref, o_ref = xin.at[slot], xout.at[slot]
        x = x0_ref[...].astype(F32)
        for l in range(L):
            proj = jnp.dot(x.astype(w_ref.dtype), w_ref[l], preferred_element_type=F32)
            x = x0_ref[...].astype(F32) * (proj + b_ref[l:l + 1, :].astype(F32)) + x
        for j in range(out_parts):
            cols = part(j, out_parts)
            o_ref[:, cols] = x[:, cols].astype(o_ref.dtype)
            pltpu.make_async_copy(o_ref.at[:, cols], o_hbm.at[rows(t), cols],
                                  osem.at[slot]).start()

    head_out.wait()
    out_wait(0)
    out_wait(1)


def _cross_network(x0, ws, bs, tm=512, head=512, w0_parts=4, out_parts=4, flags=None):
    B, D = x0.shape
    L = ws.shape[0]
    assert (B - head) % tm == 0 and B - head >= 2 * tm and L >= 2
    return pl.pallas_call(
        functools.partial(_kernel, out_parts=out_parts),
        in_specs=[pl.BlockSpec(memory_space=pl.ANY),
                  pl.BlockSpec(memory_space=pl.ANY),
                  pl.BlockSpec(memory_space=pltpu.VMEM)],
        out_specs=pl.BlockSpec(memory_space=pl.ANY),
        out_shape=jax.ShapeDtypeStruct((B, D), x0.dtype),
        scratch_shapes=[pltpu.VMEM((L, D, D), ws.dtype),
                        pltpu.VMEM((2, tm, D), x0.dtype),
                        pltpu.VMEM((2, tm, D), x0.dtype),
                        pltpu.VMEM((head, D), x0.dtype),
                        pltpu.VMEM((head, D), F32),
                        pltpu.SemaphoreType.DMA((L,)),
                        pltpu.SemaphoreType.DMA((w0_parts,)),
                        pltpu.SemaphoreType.DMA((2,)),
                        pltpu.SemaphoreType.DMA((2,)),
                        pltpu.SemaphoreType.DMA((2,))],
        compiler_params=pltpu.CompilerParams(vmem_limit_bytes=64 * 2**20, flags=flags),
    )(x0, ws, bs)


@jax.jit
def pallas_standalone__cross_network_dcn__recsys_kernel(x0, ws, bs):
    return _cross_network(x0, ws, bs)
```
